```python
import os as _os
_os.environ.setdefault("JAX_PLATFORMS", "cpu")
import jax
import jax.numpy as jnp

def _softmax(x, axis=-1):
    return jax.nn.softmax(x, axis=axis)
def _gelu(x):
    return jax.nn.gelu(x, approximate=True)
def _silu(x):
    return jax.nn.silu(x)
def _sigmoid(x):
    return jax.nn.sigmoid(x)
def _layernorm(x, axis=-1, eps=1e-5):
    m = jnp.mean(x, axis=axis, keepdims=True)
    v = jnp.var(x, axis=axis, keepdims=True)
    return (x - m) / jnp.sqrt(v + eps)
def _scatter_add(tgt, idx, src, axis=0):
    return tgt.at[idx].add(src)
def _segment_sum(src, seg, n):
    return jax.ops.segment_sum(src, seg, n)
class _Rng:
    def __init__(self, key):
        self._k = key
    def _next(self):
        self._k, sub = jax.random.split(self._k)
        return sub
    def normal(self, shape):
        return jax.random.normal(self._next(), shape, dtype=jnp.bfloat16)
    def randint(self, lo, hi, shape):
        return jax.random.randint(self._next(), shape, lo, hi, dtype=jnp.int32)
    def uniform(self, shape, lo=0.0, hi=1.0):
        return jax.random.uniform(self._next(), shape, jnp.bfloat16, lo, hi)
    def permutation(self, n):
        return jax.random.permutation(self._next(), n)


kernel_name = 'interleave_layers__sliding_local_dilated__softmax_full_mha__prompt'

def setup_inputs():
    _rng = _Rng(jax.random.key(int.from_bytes(__import__("os").urandom(4), "little")))
    _w = (lambda a: (lambda t: t.astype(jnp.bfloat16) if jnp.issubdtype(t.dtype, jnp.floating) else t)(jnp.asarray(a)))
    def _A_setup():
        B, S, D = 1, 2048, 512
        return {
            "x": _w((lambda *s: _rng.normal(s) * 0.05)(B, S, D)),
            "wqkv": _w((lambda *s: _rng.normal(s) * 0.05)(D, 3 * D)),
            "wo": _w((lambda *s: _rng.normal(s) * 0.05)(D, D)),
        }
    _A_in = _A_setup()

    def _B_setup():
        B, S, D = 1, 2048, 512
        return {
            "x": _w((lambda *s: _rng.normal(s) * 0.05)(B, S, D)),
            "wqkv": _w((lambda *s: _rng.normal(s) * 0.05)(D, 3 * D)),
            "wo": _w((lambda *s: _rng.normal(s) * 0.05)(D, D)),
        }
    _B_in = _B_setup()

    return {
        "A_x": _A_in["x"],
        "A_wqkv": _A_in["wqkv"],
        "A_wo": _A_in["wo"],
        "B_x": _B_in["x"],
        "B_wqkv": _B_in["wqkv"],
        "B_wo": _B_in["wo"],
    }

def reference(A_x, A_wqkv, A_wo, B_x, B_wqkv, B_wo):
    def _A_ref(x, wqkv, wo):
        B, S, D = x.shape
        H = 32; Dh = D // H
        W, dil = 8, 2
        qkv = (lambda x, *d: x.transpose(*d))((x @ wqkv).reshape(B, S, 3, H, Dh), 2, 0, 3, 1, 4)
        q, k, v = qkv[0], qkv[1], qkv[2]
        scale = Dh ** -0.5
        pos = jnp.arange(S)
        off = jnp.arange(W) * dil
        idx = pos[:, None] - off[None, :]
        mask = idx >= 0
        idx_c = jnp.where(mask, idx, 0).reshape(-1)
        kg = k[:, :, idx_c, :].reshape(B, H, S, W, Dh)
        vg = v[:, :, idx_c, :].reshape(B, H, S, W, Dh)
        logits = jnp.einsum("bhsd,bhswd->bhsw", q, kg) * scale
        logits = jnp.where(mask[None, None, :, :], logits, -1e9)
        attn = _softmax(logits, axis=-1)
        o = jnp.einsum("bhsw,bhswd->bhsd", attn, vg)
        return (lambda x, *d: x.transpose(*d))(o, 0, 2, 1, 3).reshape(B, S, D) @ wo

    def _B_ref(x, wqkv, wo):
        B, S, D = x.shape
        H = 32; Dh = D // H
        qkv = (lambda x, *d: x.transpose(*d))((x @ wqkv).reshape(B, S, 3, H, Dh), 2, 0, 3, 1, 4)
        q, k, v = qkv[0], qkv[1], qkv[2]
        scale = Dh ** -0.5
        scores = jnp.einsum("bhqd,bhkd->bhqk", q, k) * scale
        p = _softmax(scores, axis=-1)
        o = jnp.einsum("bhqk,bhkd->bhqd", p, v)
        return (lambda x, *d: x.transpose(*d))(o, 0, 2, 1, 3).reshape(B, S, D) @ wo

    x = A_x
    x = x + _A_ref(_layernorm(x, axis=-1), A_wqkv, A_wo)
    x = x + _B_ref(_layernorm(x, axis=-1), B_wqkv, B_wo)
    x = x + _A_ref(_layernorm(x, axis=-1), A_wqkv, A_wo)
    x = x + _B_ref(_layernorm(x, axis=-1), B_wqkv, B_wo)
    return x
```

```python
import jax
import jax.numpy as jnp
import numpy as np
from jax import lax
import jax.experimental.pallas as pl
import jax.experimental.pallas.tpu as pltpu

S, D, H, DH = 2048, 512, 32, 16
WIN, DIL = 8, 2
L = 128
NB = S // L
NF = D // L
EPS = 1e-5
LOG2E = float(np.log2(np.e))
SCALE = DH ** -0.5

NC = 4
DEPTH = 2
DOUBLE = (12, 12, 12, 12)
HPI = 2
L_MIN, L_MAX, O_MAX = 2.0 ** -60, 2.0 ** 100, 3.0e38

F32, BF16, U32 = jnp.float32, jnp.bfloat16, jnp.uint32


def _dot(a, b):
    return jnp.dot(a, b, preferred_element_type=F32)


def _words(x):
    return pltpu.bitcast(x.astype(BF16), U32)


def _halves(w):
    return pltpu.bitcast(w, BF16)


def _total(xs):
    acc = xs[0]
    for x in xs[1:]:
        acc = acc + x
    return acc


def _slot(c, row=0, n=D):
    start = c * D + row
    return pl.ds(start if isinstance(start, int) else pl.multiple_of(start, 16), n)


def _lanes(j):
    return pl.ds(j * L if isinstance(j, int) else pl.multiple_of(j * L, L), L)


def _col(j, n=1):
    return slice(j * L, (j + n) * L)


def _kernel(z_ref, x_hbm, wa_hbm, woa_hbm, wb_hbm, wob_hbm, out_hbm,
            x_io, wa_in, woa_in, wb_in, wob_in, tmp,
            xt, xn, wat, woat, wbt, wobt,
            kva, qa0, qa1, oa0, oa1,
            qw, vw, kw, ot, qf, kb0, kb1, sems):
    x_in = [pltpu.make_async_copy(x_hbm.at[:, _col(f)], x_io.at[f], sems.at[f]) for f in range(NF)]
    x_out = [pltpu.make_async_copy(x_io.at[f], out_hbm.at[:, _col(f)], sems.at[f]) for f in range(NF)]
    wa_part = [pltpu.make_async_copy(wa_hbm.at[:, _col(NF * i, NF)], wa_in.at[i], sems.at[NF + i])
               for i in range(3)]
    w_rest = [pltpu.make_async_copy(src, dst, sems.at[NF + 3 + i]) for i, (src, dst) in enumerate(
        [(woa_hbm, woa_in), (wb_hbm, wb_in), (wob_hbm, wob_in)])]
    x_pairs = x_io.bitcast(U32)

    def transpose_wa(part):
        for kc in range(NF):
            for g in range(NF):
                tmp[kc, _col(g), :] = wa_in[part, _col(kc), _col(g)].astype(F32).T
            for d in range(DH):
                row = (part * D + d * H) // 2
                wat[row:row + H // 2, _col(kc)] = _words(tmp[kc, pl.ds(d, H, stride=DH), :])

    def transpose_woa():
        for oc in range(NF):
            tmp[oc] = woa_in[:, _col(oc)].astype(F32)
            for g in range(NF):
                blk = jnp.concatenate(
                    [tmp[oc, pl.ds(d, H, stride=DH), :] for d in range(4 * g, 4 * g + 4)], axis=0)
                woat[oc * 64:(oc + 1) * 64, _col(g)] = _words(blk.T)

    def transpose_plain(w_in, wt):
        for oc in range(w_in.shape[1] // L):
            for g in range(NF):
                wt[oc * 64:(oc + 1) * 64, _col(g)] = _words(w_in[_col(g), _col(oc)].astype(F32).T)

    def after(mark, y, row=0):
        if mark is None:
            return y
        never = lax.broadcasted_iota(jnp.int32, (8, L), 1) < z_ref[0]
        tied = jnp.where(never, pltpu.bitcast(mark, y.dtype), y[row:row + 8])
        parts = [y[:row]] if row else []
        parts.append(tied)
        if row + 8 < y.shape[0]:
            parts.append(y[row + 8:])
        return jnp.concatenate(parts, axis=0)

    def project(wt, part, y):
        return _dot(_halves(wt[part * D // 2:(part + 1) * D // 2, :]), y)

    def layernorm(j):
        x = xt[:, _col(j)]
        mean = jnp.sum(x, axis=0, keepdims=True) * (1.0 / D)
        xc = x - mean
        var = jnp.sum(xc * xc, axis=0, keepdims=True) * (1.0 / D)
        return xc * lax.rsqrt(var + EPS)

    qas, oas = (qa0, qa1), (oa0, oa1)

    def layer_a_kv():
        lane0 = lax.broadcasted_iota(jnp.int32, (D, L), 1) == 0

        mark = None
        for j in range(NB):
            y = layernorm(j)
            xn[j] = _words(y)
            y = after(mark, y).astype(BF16)
            k, v = project(wat, 1, y), project(wat, 2, y)
            if j == 0:
                v_first = v
            else:
                mark = kva[_slot(z_ref[j] + NB, 0, 8), :]
            kva[_slot(NB + j), :] = k
            kva[_slot(3 * NB + j), :] = v
            if j >= DIL:
                kva[_slot(j), :] = pltpu.roll(k, 1, 1)
                kva[_slot(2 * NB + j), :] = jnp.where(lane0, v_first, pltpu.roll(v, 1, 1))
            if j == 1:
                transpose_wa(0)
        qa0[...] = project(wat, 0, _halves(xn[0]))

    def layer_a_attend():
        lane = lax.broadcasted_iota(jnp.int32, (16, L), 1)
        zeros = [pl.multiple_of(z_ref[i], 16) for i in range(NF)]

        def attend(j, par, h0):
            src = [j + NB - DIL * w for w in range(WIN)]
            logits = [None] * WIN
            for d in range(DH):
                q = qas[par][pl.ds(zeros[0] + d * H + h0, 16), :]
                for w, c in enumerate(src):
                    t = q * kva[_slot(c, d * H + h0, 16), :]
                    logits[w] = t if d == 0 else logits[w] + t
                yield logits[-1][0:8]
            for w in range(WIN):
                t = logits[w] * (SCALE * LOG2E)
                if w and not (isinstance(j, int) and j >= DIL * w):
                    t = jnp.where(lane < jnp.where(j < DIL * w, 1, 0), -1e9 * LOG2E, t)
                logits[w] = t
            m = logits[0]
            for t in logits[1:]:
                m = jnp.maximum(m, t)
            e = [jnp.exp2(t - m) for t in logits]
            inv = 1.0 / _total(e)
            p = [t * inv for t in e]
            for d in range(DH):
                o = _total([p[w] * kva[_slot(2 * NB + c, d * H + h0, 16), :] for w, c in enumerate(src)])
                oas[par][(d * H + h0) // 2:(d * H + h0) // 2 + 8, :] = _words(o)
                yield o[0:8]

        def tile_dot(wt, r, rhs, vpu):
            acc = None
            for kc in range(NF):
                w = wt[r * 64:(r + 1) * 64, _col(kc)]
                next(vpu, None)
                w = after(next(vpu, None), w, 32)
                y = _dot(_halves(w), _halves(rhs(kc, r)))
                acc = y if acc is None else acc + y
            return acc

        def step(j, par, do_q=True, do_attend=True, do_out=True):
            vpu = (x for h0 in range(0, H, 16) for x in attend(j + 1, 1 - par, h0)) if do_attend else iter(())
            if do_q:
                for r in range(NF):
                    qas[par][_col(r), :] = tile_dot(
                        wat, r, lambda kc, r: xn[j + 2, pl.ds(zeros[r] + kc * 64, 64), :], vpu)
            if do_out:
                cols = _lanes(j)
                for r in range(NF):
                    xt[_col(r), cols] = xt[_col(r), cols] + tile_dot(
                        woat, r, lambda kc, r: oas[par][pl.ds(zeros[r] + kc * 64, 64), :], vpu)
            for _ in vpu:
                pass

        step(-1, 1, do_out=False)

        def body(i, carry):
            step(2 * i, 0)
            step(2 * i + 1, 1)
            return carry

        lax.fori_loop(0, NB // 2 - 1, body, 0)
        step(NB - 2, 0, do_q=False)
        step(NB - 1, 1, do_q=False, do_attend=False)

    def layer_b_qkv():
        for j in range(NB):
            y = layernorm(j).astype(BF16)
            q32 = project(wbt, 0, y) * (SCALE * LOG2E)
            q = _words(q32)
            k = project(wbt, 1, y)
            v = _words(project(wbt, 2, y))
            for h in range(H):
                qf[h, j] = q32[DH * h:DH * h + DH]
                qw[h, j] = q[8 * h:8 * h + 8]
                vw[h, j] = v[8 * h:8 * h + 8]
            for g in range(D // L):
                kt = _words(k[_col(g)].T)
                for i in range(8):
                    kw[8 * g + i, j] = kt if i == 0 else pltpu.roll(kt, L - DH * i, 1)
            spread_k(0, j, 0)

    def q_weights(words):
        return _halves(jnp.concatenate([words, jnp.zeros((56, L), U32)], axis=0))

    def vpu_groups(e, i, j):
        return 2 if e == 1 and j >= DOUBLE[i] else 1

    def spread_k(h, j, e):
        n = vpu_groups(e, -1, j)
        k = _halves(kw[h, j, 64 - 8 * n:64, :]).astype(F32)
        for d in range(DH):
            (kb0, kb1)[e][j * DH + d, 0:16 * n, :] = jnp.broadcast_to(k[:, d:d + 1], (16 * n, L))

    def layer_b_attend_fast():
        nq = NB // NC
        steps = [(e, i, j) for e in range(HPI) for i in range(nq) for j in range(NB)]
        n = len(steps)

        def body(it, bad):
            zs = [z_ref[i] for i in range(2 * NB)]
            scores, den, acc = {}, {}, {}

            def qk(t, m):
                e, i, j = steps[t]
                h, c = it * HPI + e, i * NC + m
                order = range(7 - vpu_groups(e, i, j), -1, -1)
                lhs = jnp.concatenate([kw[h + zs[NB + c], j, 8 * u:8 * u + 8, :] for u in order], axis=0)
                s = _dot(_halves(lhs), q_weights(qw[h + zs[j], c]))
                scores[t, m] = [s[16 * u:16 * u + 16] for u in order]

            for t in range(-DEPTH, n):
                if t >= 0:
                    e, i, j = steps[t]
                    h = it * HPI + e
                    if j % nq == 0:
                        spread_k(jnp.minimum(h + 1, H - 1), (i * NB + j) // nq, 1 - e)
                for m in range(NC):
                    if t >= 0:
                        c = i * NC + m
                        part = [[] for _ in range(2 * vpu_groups(e, i, j))]
                        end = 16 * vpu_groups(e, -1, j)
                        for d in range(DH):
                            kd = (kb0, kb1)[e][zs[NB + c] + j * DH + d, end - 8 * len(part):end, :]
                            qd = qf[h + zs[j], c, pl.ds(d, 8, stride=0), :]
                            for r in range(len(part)):
                                part[r].append(kd[8 * r:8 * r + 8] * qd)
                        rows = scores.pop((t, m)) + [jnp.concatenate([_total(x) for x in part], axis=0)]
                        p = jnp.concatenate([jnp.exp2(x) for x in rows], axis=0)
                        ls = _total([p[r:r + 8] + p[r + 8:r + 16] for r in range(L - 16, -8, -16)])
                        pt = p.astype(BF16)
                    if t + DEPTH < n:
                        qk(t + DEPTH, m)
                    if t >= 0:
                        a = _dot(_halves(vw[h + zs[NB + c], j]), pt)
                        acc[c] = a if j == 0 else acc[c] + a
                        den[c] = ls if j == 0 else den[c] + ls
                        if j == NB - 1:
                            l = jnp.sum(den[c], axis=0, keepdims=True)
                            ok = (l >= L_MIN) & (l <= L_MAX) & (jnp.abs(acc[c]) <= O_MAX)
                            bad = jnp.maximum(bad, jnp.where(ok, 0.0, 1.0))
                            ot[c, h] = _words(acc[c] * (1.0 / l))
            return bad

        return jnp.max(lax.fori_loop(0, H // HPI, body, jnp.zeros((DH, L), F32)))

    def layer_b_attend_exact():
        def body(it, carry):
            h, c = it // NB, it % NB
            k = _halves(kw[h].reshape(NB * 64, L))
            s = _dot(k, q_weights(qw[h, c]))
            p = jnp.exp2(s - jnp.max(s, axis=0, keepdims=True))
            l = jnp.sum(p, axis=0, keepdims=True)
            v = jnp.concatenate([_halves(vw[h, j]) for j in range(NB)], axis=1)
            ot[c, h] = _words(_dot(v, p.astype(BF16)) * (1.0 / l))
            return carry

        lax.fori_loop(0, H * NB, body, 0)

    def heads_out(j):
        return _halves(ot[j].reshape(H * 8, L))

    def layer_b_out():
        for j in range(NB):
            xt[:, _col(j)] = xt[:, _col(j)] + project(wobt, 0, heads_out(j))

    def layer_b_out_final():
        def bits(f, j):
            y = xt[_col(f), _col(j)] + _dot(_halves(wobt[f * 64:(f + 1) * 64, :]), heads_out(j))
            return pltpu.bitcast(y.astype(BF16).astype(F32), U32)

        for f in range(NF):
            for jj in range(NB // 2):
                pair = (bits(f, 2 * jj) >> 16) | bits(f, 2 * jj + 1)
                x_pairs[f, pl.ds(jj, L, stride=NB // 2), :] = pair.T
            x_out[f].start()
        for c in x_out:
            c.wait()

    wa_part[1].start()
    wa_part[2].start()
    wa_part[1].wait()
    for c in x_in:
        c.start()
    transpose_wa(1)
    wa_part[2].wait()
    wa_part[0].start()
    transpose_wa(2)
    for f in range(NF):
        x_in[f].wait()
        if f == NF - 1:
            for c in w_rest:
                c.start()
        for jj in range(NB // 2):
            pair = x_pairs[f, pl.ds(jj, L, stride=NB // 2), :].T
            xt[_col(f), _col(2 * jj)] = pltpu.bitcast(pair << 16, F32)
            xt[_col(f), _col(2 * jj + 1)] = pltpu.bitcast(pair & np.uint32(0xFFFF0000), F32)
    wa_part[0].wait()

    def layer_pair(it, carry):
        layer_a_kv()

        @pl.when(it == 0)
        def _():
            for c in w_rest:
                c.wait()
            transpose_woa()

        layer_a_attend()
        transpose_plain(wb_in, wbt)
        transpose_plain(wob_in, wobt)
        layer_b_qkv()
        redo = layer_b_attend_fast()
        pl.when(redo > 0.0)(layer_b_attend_exact)
        pl.when(it == 0)(layer_b_out)
        return carry

    lax.fori_loop(0, 2, layer_pair, 0)
    layer_b_out_final()


@jax.jit
def pallas_interleave_layers__sliding_local_dilated__softmax_full_mha__prompt_kernel(
    A_x: jax.Array,
    A_wqkv: jax.Array,
    A_wo: jax.Array,
    B_x: jax.Array,
    B_wqkv: jax.Array,
    B_wo: jax.Array,
):
    del B_x
    vmem = pltpu.VMEM
    scratch = (
        [vmem((NF, S, L), BF16), vmem((3, D, D), BF16), vmem((D, D), BF16),
         vmem((D, 3 * D), BF16), vmem((D, D), BF16), vmem((NF, D, L), F32),
         vmem((D, S), F32), vmem((NB, D // 2, L), U32)]
        + [vmem((3 * D // 2, D), U32), vmem((D // 2, D), U32)] * 2
        + [vmem((4 * NB * D, L), F32)]
        + [vmem((D, L), F32)] * 2 + [vmem((D // 2, L), U32)] * 2
        + [vmem((H, NB, 8, L), U32)] * 2
        + [vmem((H, NB, 64, L), U32), vmem((NB, H, 8, L), U32),
           vmem((H, NB, DH, L), F32)]
        + [vmem((NB * DH, 16, L), F32), vmem((NB * DH, 32, L), F32)]
        + [pltpu.SemaphoreType.DMA((NF + 6,))])
    hbm = pl.BlockSpec(memory_space=pl.ANY)
    out = pl.pallas_call(
        _kernel,
        out_shape=jax.ShapeDtypeStruct((S, D), BF16),
        in_specs=[pl.BlockSpec(memory_space=pltpu.SMEM), hbm, hbm, hbm, hbm, hbm],
        out_specs=hbm,
        scratch_shapes=scratch,
        compiler_params=pltpu.CompilerParams(
            vmem_limit_bytes=100 * 2 ** 20,
            flags={"XLA_TPU_EVENLY_DISTRIBUTE_CRITICAL_NODES": True}),
    )(np.zeros((2 * NB,), np.int32), A_x.reshape(S, D), A_wqkv, A_wo, B_wqkv, B_wo)
    return out.reshape(A_x.shape)
```
